```python
import os as _os
_os.environ.setdefault("JAX_PLATFORMS", "cpu")
import jax
import jax.numpy as jnp

def _softmax(x, axis=-1):
    return jax.nn.softmax(x, axis=axis)
def _gelu(x):
    return jax.nn.gelu(x, approximate=True)
def _silu(x):
    return jax.nn.silu(x)
def _sigmoid(x):
    return jax.nn.sigmoid(x)
def _layernorm(x, axis=-1, eps=1e-5):
    m = jnp.mean(x, axis=axis, keepdims=True)
    v = jnp.var(x, axis=axis, keepdims=True)
    return (x - m) / jnp.sqrt(v + eps)
def _scatter_add(tgt, idx, src, axis=0):
    return tgt.at[idx].add(src)
def _segment_sum(src, seg, n):
    return jax.ops.segment_sum(src, seg, n)
class _Rng:
    def __init__(self, key):
        self._k = key
    def _next(self):
        self._k, sub = jax.random.split(self._k)
        return sub
    def normal(self, shape):
        return jax.random.normal(self._next(), shape, dtype=jnp.bfloat16)
    def randint(self, lo, hi, shape):
        return jax.random.randint(self._next(), shape, lo, hi, dtype=jnp.int32)
    def uniform(self, shape, lo=0.0, hi=1.0):
        return jax.random.uniform(self._next(), shape, jnp.bfloat16, lo, hi)
    def permutation(self, n):
        return jax.random.permutation(self._next(), n)


kernel_name = 'standalone__mha_softmax__near_ridge'

def setup_inputs():
    _rng = _Rng(jax.random.key(int.from_bytes(__import__("os").urandom(4), "little")))
    _w = (lambda a: (lambda t: t.astype(jnp.bfloat16) if jnp.issubdtype(t.dtype, jnp.floating) else t)(jnp.asarray(a)))
    B, H, Sq, Sk, D = 8, 32, 496, 512, 192
    return {
        "q": _w((lambda *s: _rng.normal(s) * 0.05)(B, H, Sq, D)),
        "k": _w((lambda *s: _rng.normal(s) * 3.2)(B, H, Sk, D)),
        "v": _w((lambda *s: _rng.normal(s) * 0.05)(B, H, Sk, D)),
    }

def reference(q, k, v):
    scale = q.shape[-1] ** -0.5
    scores = jnp.einsum("bhqd,bhkd->bhqk", q, k) * scale
    p = _softmax(scores, axis=-1)
    return jnp.einsum("bhqk,bhkd->bhqd", p, v)
```

```python
import functools

import jax
import jax.numpy as jnp
import jax.experimental.pallas as pl
import jax.experimental.pallas.tpu as pltpu


def _mha_kernel(q_ref, k_ref, v_ref, o_ref, *, heads_per_step, scale):
    def one_head(h, carry):
        q = q_ref[h]
        k = k_ref[h]
        v = v_ref[h]
        s = jax.lax.dot_general(
            q, k, (((1,), (1,)), ((), ())), preferred_element_type=jnp.float32
        ) * scale
        m = jnp.max(s, axis=-1, keepdims=True)
        p = jnp.exp(s - m)
        l = jnp.sum(p, axis=-1, keepdims=True)
        o = jnp.dot(p.astype(jnp.bfloat16), v, preferred_element_type=jnp.float32)
        o_ref[h] = (o * (1.0 / l)).astype(o_ref.dtype)
        return carry

    jax.lax.fori_loop(0, heads_per_step, one_head, 0)


@jax.jit
def pallas_standalone__mha_softmax__near_ridge_kernel(
    q: jax.Array,
    k: jax.Array,
    v: jax.Array,
):
    B, H, Sq, D = q.shape
    Sk = k.shape[2]
    BH = B * H
    q3 = q.reshape(BH, Sq, D)
    k3 = k.reshape(BH, Sk, D)
    v3 = v.reshape(BH, Sk, D)
    hps = 4
    assert BH % hps == 0
    scale = float(D) ** -0.5

    out = pl.pallas_call(
        functools.partial(_mha_kernel, heads_per_step=hps, scale=scale),
        grid=(BH // hps,),
        in_specs=[
            pl.BlockSpec((hps, Sq, D), lambda i: (i, 0, 0)),
            pl.BlockSpec((hps, Sk, D), lambda i: (i, 0, 0)),
            pl.BlockSpec((hps, Sk, D), lambda i: (i, 0, 0)),
        ],
        out_specs=pl.BlockSpec((hps, Sq, D), lambda i: (i, 0, 0)),
        out_shape=jax.ShapeDtypeStruct((BH, Sq, D), q.dtype),
        compiler_params=pltpu.CompilerParams(
            dimension_semantics=("parallel",),
            vmem_limit_bytes=64 * 1024 * 1024,
        ),
    )(q3, k3, v3)
    return out.reshape(B, H, Sq, D)
```

```python
import functools
import math

import jax
import jax.numpy as jnp
import jax.experimental.pallas as pl
import jax.experimental.pallas.tpu as pltpu

HPS = 8

def _mha_kernel(q_ref, k_ref, v_ref, o_ref, s_ref, *, heads_per_step, c2):
    def qk(h, slot):
        s_ref[slot] = jax.lax.dot_general(
            k_ref[h], q_ref[h], (((0,), (0,)), ((), ())),
            preferred_element_type=jnp.float32)

    def sm_pv(h, slot):
        sT = s_ref[slot]
        m = jnp.max(sT, axis=0, keepdims=True)
        pT = jnp.exp2(sT * c2 - m * c2)
        l = jnp.sum(pT, axis=0, keepdims=True)
        oT = jnp.dot(v_ref[h], pT.astype(jnp.bfloat16), preferred_element_type=jnp.float32)
        o_ref[h] = (oT * (1.0 / l)).astype(o_ref.dtype)

    qk(0, 0)
    for h in range(heads_per_step):
        if h + 1 < heads_per_step:
            qk(h + 1, (h + 1) % 2)
        sm_pv(h, h % 2)


@jax.jit
def pallas_standalone__mha_softmax__near_ridge_kernel(
    q: jax.Array,
    k: jax.Array,
    v: jax.Array,
):
    B, H, Sq, D = q.shape
    Sk = k.shape[2]
    BH = B * H
    qT = jnp.swapaxes(q, 2, 3).reshape(BH, D, Sq)
    kT = jnp.swapaxes(k, 2, 3).reshape(BH, D, Sk)
    vT = jnp.swapaxes(v, 2, 3).reshape(BH, D, Sk)
    hps = HPS
    assert BH % hps == 0
    c2 = float(D) ** -0.5 * math.log2(math.e)

    outT = pl.pallas_call(
        functools.partial(_mha_kernel, heads_per_step=hps, c2=c2),
        grid=(BH // hps,),
        in_specs=[
            pl.BlockSpec((hps, D, Sq), lambda i: (i, 0, 0)),
            pl.BlockSpec((hps, D, Sk), lambda i: (i, 0, 0)),
            pl.BlockSpec((hps, D, Sk), lambda i: (i, 0, 0)),
        ],
        out_specs=pl.BlockSpec((hps, D, Sq), lambda i: (i, 0, 0)),
        out_shape=jax.ShapeDtypeStruct((BH, D, Sq), q.dtype),
        scratch_shapes=[pltpu.VMEM((2, Sk, Sq), jnp.float32)],
        compiler_params=pltpu.CompilerParams(
            dimension_semantics=("parallel",),
            vmem_limit_bytes=64 * 1024 * 1024,
        ),
    )(qT, kT, vT)
    return jnp.swapaxes(outT.reshape(B, H, D, Sq), 2, 3)
```

```python
import functools
import math

import jax
import jax.numpy as jnp
import jax.experimental.pallas as pl
import jax.experimental.pallas.tpu as pltpu

HPS = 8

def _mha_kernel(q_ref, k_ref, v_ref, o_ref, s_ref, m_ref, *, heads_per_step, c2):
    def qk(h, slot):
        s = jax.lax.dot_general(
            k_ref[h], q_ref[h], (((0,), (0,)), ((), ())),
            preferred_element_type=jnp.float32)
        s_ref[slot] = s
        m_ref[slot] = jnp.max(s, axis=0, keepdims=True) * c2

    def sm_pv(h, slot):
        sT = s_ref[slot]
        pT = jnp.exp2(sT * c2 - m_ref[slot])
        l = jnp.sum(pT, axis=0, keepdims=True)
        oT = jnp.dot(v_ref[h], pT.astype(jnp.bfloat16), preferred_element_type=jnp.float32)
        o_ref[h] = (oT * (1.0 / l)).astype(o_ref.dtype)

    qk(0, 0)
    for h in range(heads_per_step):
        if h + 1 < heads_per_step:
            qk(h + 1, (h + 1) % 2)
        sm_pv(h, h % 2)


@jax.jit
def pallas_standalone__mha_softmax__near_ridge_kernel(
    q: jax.Array,
    k: jax.Array,
    v: jax.Array,
):
    B, H, Sq, D = q.shape
    Sk = k.shape[2]
    BH = B * H
    qT = jnp.swapaxes(q, 2, 3).reshape(BH, D, Sq)
    kT = jnp.swapaxes(k, 2, 3).reshape(BH, D, Sk)
    vT = jnp.swapaxes(v, 2, 3).reshape(BH, D, Sk)
    hps = HPS
    assert BH % hps == 0
    c2 = float(D) ** -0.5 * math.log2(math.e)

    outT = pl.pallas_call(
        functools.partial(_mha_kernel, heads_per_step=hps, c2=c2),
        grid=(BH // hps,),
        in_specs=[
            pl.BlockSpec((hps, D, Sq), lambda i: (i, 0, 0)),
            pl.BlockSpec((hps, D, Sk), lambda i: (i, 0, 0)),
            pl.BlockSpec((hps, D, Sk), lambda i: (i, 0, 0)),
        ],
        out_specs=pl.BlockSpec((hps, D, Sq), lambda i: (i, 0, 0)),
        out_shape=jax.ShapeDtypeStruct((BH, D, Sq), q.dtype),
        scratch_shapes=[pltpu.VMEM((2, Sk, Sq), jnp.float32), pltpu.VMEM((2, 1, Sq), jnp.float32)],
        compiler_params=pltpu.CompilerParams(
            dimension_semantics=("parallel",),
            vmem_limit_bytes=64 * 1024 * 1024,
        ),
    )(qT, kT, vT)
    return jnp.swapaxes(outT.reshape(B, H, D, Sq), 2, 3)
```
